```python
import os as _os
_os.environ.setdefault("JAX_PLATFORMS", "cpu")
import jax
import jax.numpy as jnp

def _softmax(x, axis=-1):
    return jax.nn.softmax(x, axis=axis)
def _gelu(x):
    return jax.nn.gelu(x, approximate=True)
def _silu(x):
    return jax.nn.silu(x)
def _sigmoid(x):
    return jax.nn.sigmoid(x)
def _layernorm(x, axis=-1, eps=1e-5):
    m = jnp.mean(x, axis=axis, keepdims=True)
    v = jnp.var(x, axis=axis, keepdims=True)
    return (x - m) / jnp.sqrt(v + eps)
def _scatter_add(tgt, idx, src, axis=0):
    return tgt.at[idx].add(src)
def _segment_sum(src, seg, n):
    return jax.ops.segment_sum(src, seg, n)
class _Rng:
    def __init__(self, key):
        self._k = key
    def _next(self):
        self._k, sub = jax.random.split(self._k)
        return sub
    def normal(self, shape):
        return jax.random.normal(self._next(), shape, dtype=jnp.bfloat16)
    def randint(self, lo, hi, shape):
        return jax.random.randint(self._next(), shape, lo, hi, dtype=jnp.int32)
    def uniform(self, shape, lo=0.0, hi=1.0):
        return jax.random.uniform(self._next(), shape, jnp.bfloat16, lo, hi)
    def permutation(self, n):
        return jax.random.permutation(self._next(), n)


kernel_name = 'parallel_sum__softmax_full_mha__moe_arch_mod__prompt'

def setup_inputs():
    _rng = _Rng(jax.random.key(int.from_bytes(__import__("os").urandom(4), "little")))
    _w = (lambda a: (lambda t: t.astype(jnp.bfloat16) if jnp.issubdtype(t.dtype, jnp.floating) else t)(jnp.asarray(a)))
    def _A_setup():
        B, S, D = 1, 2048, 512
        return {
            "x": _w((lambda *s: _rng.normal(s) * 0.05)(B, S, D)),
            "wqkv": _w((lambda *s: _rng.normal(s) * 0.1)(D, 3 * D)),
            "wo": _w((lambda *s: _rng.normal(s) * 0.05)(D, D)),
        }
    _A_in = _A_setup()

    def _B_setup():
        B, S, D, F, C = 1, 2048, 512, 1792, 1
        return {
            "x": _w((lambda *s: _rng.normal(s) * 0.05)(B, S, D)),
            "w_r": _w((lambda *s: _rng.normal(s) * 1.6)(D)),
            "w_gate": _w((lambda *s: _rng.normal(s) * 0.1)(D, F)),
            "w_up": _w((lambda *s: _rng.normal(s) * 0.1)(D, F)),
            "w_down": _w((lambda *s: _rng.normal(s) * 0.1)(F, D)),
        }
    _B_in = _B_setup()

    return {
        "A_x": _A_in["x"],
        "A_wqkv": _A_in["wqkv"],
        "A_wo": _A_in["wo"],
        "B_x": _B_in["x"],
        "B_w_r": _B_in["w_r"],
        "B_w_gate": _B_in["w_gate"],
        "B_w_up": _B_in["w_up"],
        "B_w_down": _B_in["w_down"],
    }

def reference(A_x, A_wqkv, A_wo, B_x, B_w_r, B_w_gate, B_w_up, B_w_down):
    def _A_ref(x, wqkv, wo):
        B, S, D = x.shape
        H = 32; Dh = D // H
        qkv = (lambda x, *d: x.transpose(*d))((x @ wqkv).reshape(B, S, 3, H, Dh), 2, 0, 3, 1, 4)
        q, k, v = qkv[0], qkv[1], qkv[2]
        scale = Dh ** -0.5
        scores = jnp.einsum("bhqd,bhkd->bhqk", q, k) * scale
        p = _softmax(scores, axis=-1)
        o = jnp.einsum("bhqk,bhkd->bhqd", p, v)
        return (lambda x, *d: x.transpose(*d))(o, 0, 2, 1, 3).reshape(B, S, D) @ wo

    def _B_ref(x, w_r, w_gate, w_up, w_down):
        B, S, D = x.shape
        C = 1
        r = x @ w_r
        idx = jnp.argsort(-r, axis=-1)[:, :C]
        idx_e = jnp.repeat(idx.reshape(B, C, 1), D, axis=2)
        x_sel = jnp.take_along_axis(x, idx_e, axis=1)
        g = _silu(x_sel @ w_gate)
        u = x_sel @ w_up
        y = (g * u) @ w_down
        r_sel = _sigmoid(jnp.take_along_axis(r, idx, axis=1))
        y = y * r_sel.reshape(B, C, 1)
        b_off = (jnp.arange(B) * S).reshape(B, 1)
        flat_idx = (idx + b_off).reshape(B * C)
        zero = (x * 0.0).reshape(B * S, D)
        upd = _scatter_add(zero, flat_idx, y.reshape(B * C, D), axis=0)
        return x + upd.reshape(B, S, D)

    x = A_x
    xn = _layernorm(x, axis=-1)
    return x + _A_ref(xn, A_wqkv, A_wo) + _B_ref(xn, B_w_r, B_w_gate, B_w_up, B_w_down)
```

```python
import numpy as np
import jax
import jax.numpy as jnp
from jax import lax
import jax.experimental.pallas as pl
import jax.experimental.pallas.tpu as pltpu

S = 2048
D = 512
H = 32
DH = D // H
F = 1792

QB = 512
NQ = S // QB
CH = 128
NC = S // CH
RB = 512
NR = S // RB
HG = 128 // DH
WROWS = 2 * D + 16

F32 = jnp.float32
BF16 = jnp.bfloat16
QSCALE = float(DH ** -0.5 * np.log2(np.e))
EPS_BF16 = float(np.asarray(1e-5, dtype=np.float32).astype(jnp.bfloat16).astype(np.float32))


def _rb(v):
    return v.astype(BF16).astype(F32)


def _kernel(x_hbm, w_hbm, wo_hbm, wr_hbm, wg_hbm, wu_hbm, wd_hbm, out_hbm,
            x_s, w_s, wo_s, wr_s, wg_s, wu_s, wd_s,
            xn_s, xr_s, wt_s, k_s, qt_s, vt_s, r_s, ot_s, out_s,
            sems, osems, *bufs):
    sa, sb = bufs[0:NQ], bufs[NQ:2 * NQ]
    ma, mb = bufs[2 * NQ:3 * NQ], bufs[3 * NQ:4 * NQ]

    cx = [pltpu.make_async_copy(x_hbm.at[pl.ds(i * RB, RB)], x_s.at[pl.ds(i * RB, RB)], sems.at[i])
          for i in range(NR)]
    cw = pltpu.make_async_copy(w_hbm, w_s, sems.at[NR])
    cwr = pltpu.make_async_copy(wr_hbm, wr_s, sems.at[NR + 1])
    cwo = pltpu.make_async_copy(wo_hbm, wo_s, sems.at[NR + 2])
    cwg = pltpu.make_async_copy(wg_hbm, wg_s, sems.at[NR + 3])
    cwu = pltpu.make_async_copy(wu_hbm, wu_s, sems.at[NR + 4])
    cwd = pltpu.make_async_copy(wd_hbm, wd_s, sems.at[NR + 5])
    cw.start()
    cwr.start()
    for c in cx:
        c.start()

    cw.wait()
    cwr.wait()
    wt_s[0:D, :] = w_s[:, 0:D].T
    wt_s[D:2 * D, :] = w_s[:, 2 * D:3 * D].T
    wrow = lax.broadcasted_iota(jnp.int32, (16, D), 0)
    wr_f = jnp.broadcast_to(wr_s[...].astype(F32), (16, D))
    wt_s[2 * D:WROWS, :] = jnp.where(wrow == 0, wr_f, 0.0).astype(BF16)

    for i in range(NR):
        cx[i].wait()
        rows = slice(i * RB, (i + 1) * RB)
        xf = x_s[rows, :].astype(F32)
        mean = jnp.sum(xf, axis=1, keepdims=True) * (1.0 / D)
        cen = xf - mean
        var = jnp.sum(cen * cen, axis=1, keepdims=True) * (1.0 / D)
        sd = _rb(jnp.sqrt(_rb(_rb(var) + EPS_BF16)))
        xn = (_rb(xf - _rb(mean)) / sd).astype(BF16)
        xn_s[rows, :] = xn
        xr_s[rows, :] = xf + xn.astype(F32)

    cwo.start()
    cwg.start()
    cwu.start()
    cwd.start()

    def proj(i, carry):
        rows = pl.ds(pl.multiple_of(i * RB, RB), RB)
        xn = xn_s[rows, :]
        k = jnp.dot(xn, w_s[:, D:2 * D], preferred_element_type=F32).astype(BF16)
        for g in range(D // 128):
            k_s[g, rows, :] = k[:, g * 128:(g + 1) * 128]
        t = lax.dot_general(wt_s[...], xn, (((1,), (1,)), ((), ())), preferred_element_type=F32)
        qt_s[:, rows] = (t[0:D] * QSCALE).astype(BF16)
        vt_s[:, rows] = t[D:2 * D].astype(BF16)
        r_s[:, rows] = t[2 * D:2 * D + 8]
        return carry

    lax.fori_loop(0, NR, proj, 0)

    r = _rb(r_s[0:1, :])
    r = jnp.where(r != r, -jnp.inf, r)
    rmax = jnp.max(r, axis=1, keepdims=True)
    pos = lax.broadcasted_iota(jnp.int32, (1, S), 1)
    idx = jnp.min(jnp.where(r == rmax, pos, S - 1), axis=1, keepdims=True)
    idx_s = idx[0, 0]
    base = pl.multiple_of((idx_s // 16) * 16, 16)
    sel = lax.broadcasted_iota(jnp.int32, (16, D), 0) == (idx_s - base)
    xsel = jnp.where(sel, xn_s[pl.ds(base, 16), :].astype(F32), 0.0).astype(BF16)
    cwg.wait()
    cwu.wait()
    cwd.wait()
    gate = jnp.dot(xsel, wg_s[...], preferred_element_type=F32)
    up = jnp.dot(xsel, wu_s[...], preferred_element_type=F32)
    act = (gate * jax.nn.sigmoid(gate) * up).astype(BF16)
    y = jnp.dot(act, wd_s[...], preferred_element_type=F32)
    y = y * jax.nn.sigmoid(rmax)
    xr_s[pl.ds(base, 16), :] += jnp.where(sel, y, 0.0)

    def step(x, h1, s1, m1, h2, s2, m2):
        qs = slice(x * QB, (x + 1) * QB)
        if h1 is not None:
            g = h1 // HG
            q = pltpu.bitcast(qt_s[pl.ds(pl.multiple_of(g * 128, 128), 128), qs], jnp.uint32)
            row = lax.broadcasted_iota(jnp.int32, q.shape, 0)
            q = jnp.where((row >> 3) == h1 % HG, q, jnp.zeros_like(q))
            qm = pltpu.bitcast(q, BF16)
            mx = None
        if h2 is not None:
            m = m2[...]
            hrows = pl.ds(pl.multiple_of(h2 * DH, DH), DH)
            o = None
            l = None
        for c in range(NC):
            ks = slice(c * CH, (c + 1) * CH)
            if h1 is not None:
                s = jnp.dot(k_s[g, ks, :], qm, preferred_element_type=F32)
                s1[ks, :] = s
                cm = jnp.max(s.reshape(CH // 8, 8, QB), axis=0)
                mx = cm if mx is None else jnp.maximum(mx, cm)
            if h2 is not None:
                p = jnp.exp2(s2[ks, :] - m)
                cl = None
                for j in reversed(range(CH // 8)):
                    pj = p[j * 8:(j + 1) * 8, :]
                    cl = pj if cl is None else cl + pj
                l = cl if l is None else l + cl
                co = jnp.dot(vt_s[hrows, ks], p.astype(BF16), preferred_element_type=F32)
                o = co if o is None else o + co
        if h1 is not None:
            m1[...] = jnp.max(mx, axis=0, keepdims=True)
        if h2 is not None:
            ot_s[hrows, qs] = (o / jnp.sum(l, axis=0, keepdims=True)).astype(BF16)

    for x in range(NQ):
        step(x, 0, sa[x], ma[x], None, None, None)

    def head(i, carry):
        @pl.when(i % 2 == 0)
        def _():
            for x in range(NQ):
                step(x, i + 1, sb[x], mb[x], i, sa[x], ma[x])

        @pl.when(i % 2 == 1)
        def _():
            for x in range(NQ):
                step(x, i + 1, sa[x], ma[x], i, sb[x], mb[x])

        return carry

    lax.fori_loop(0, H - 1, head, 0)

    cwo.wait()
    co = []
    for x in range(NQ):
        step(x, None, None, None, H - 1, sb[x], mb[x])
        qs = slice(x * QB, (x + 1) * QB)
        a = lax.dot_general(ot_s[:, qs], wo_s[...], (((0,), (0,)), ((), ())), preferred_element_type=F32)
        out_s[qs, :] = (a + xr_s[qs, :]).astype(BF16)
        cp = pltpu.make_async_copy(out_s.at[pl.ds(x * QB, QB)], out_hbm.at[pl.ds(x * QB, QB)], osems.at[x])
        cp.start()
        co.append(cp)
    for cp in co:
        cp.wait()


@jax.jit
def pallas_parallel_sum__softmax_full_mha__moe_arch_mod__prompt_kernel(
    A_x: jax.Array,
    A_wqkv: jax.Array,
    A_wo: jax.Array,
    B_x: jax.Array,
    B_w_r: jax.Array,
    B_w_gate: jax.Array,
    B_w_up: jax.Array,
    B_w_down: jax.Array,
):
    del B_x
    any_spec = pl.BlockSpec(memory_space=pl.ANY)
    vmem = pltpu.VMEM
    scratch = [
        vmem((S, D), BF16),
        vmem((D, 3 * D), BF16),
        vmem((D, D), BF16),
        vmem((1, D), BF16),
        vmem((D, F), BF16),
        vmem((D, F), BF16),
        vmem((F, D), BF16),
        vmem((S, D), BF16),
        vmem((S, D), F32),
        vmem((WROWS, D), BF16),
        vmem((D // 128, S, 128), BF16),
        vmem((D, S), BF16),
        vmem((D, S), BF16),
        vmem((8, S), F32),
        vmem((D, S), BF16),
        vmem((S, D), BF16),
        pltpu.SemaphoreType.DMA((NR + 6,)),
        pltpu.SemaphoreType.DMA((NQ,)),
    ]
    scratch += [vmem((S, QB), F32)] * (2 * NQ)
    scratch += [vmem((1, QB), F32)] * (2 * NQ)
    out = pl.pallas_call(
        _kernel,
        out_shape=jax.ShapeDtypeStruct((S, D), A_x.dtype),
        in_specs=[any_spec] * 7,
        out_specs=any_spec,
        scratch_shapes=scratch,
        compiler_params=pltpu.CompilerParams(vmem_limit_bytes=100 * 1024 * 1024),
    )(A_x.reshape(S, D), A_wqkv, A_wo, B_w_r.reshape(1, D), B_w_gate, B_w_up, B_w_down)
    return out.reshape(1, S, D)
```

```python
import numpy as np
import jax
import jax.numpy as jnp
from jax import lax
import jax.experimental.pallas as pl
import jax.experimental.pallas.tpu as pltpu

S = 2048
D = 512
H = 32
DH = D // H
F = 1792

QB = 512
NQ = S // QB
CH = 128
NC = S // CH
RB = 256
NR = S // RB
HG = 128 // DH
FB = 128
NF = F // FB
T0 = 8
WROWS = 2 * D + 16

F32 = jnp.float32
BF16 = jnp.bfloat16
QSCALE = float(DH ** -0.5 * np.log2(np.e))
EPS_BF16 = float(np.asarray(1e-5, dtype=np.float32).astype(jnp.bfloat16).astype(np.float32))


def _rb(v):
    return v.astype(BF16).astype(F32)


def _kernel(x_hbm, w_hbm, wo_hbm, wr_hbm, wg_hbm, wu_hbm, wd_hbm, out_hbm,
            x_s, w_s, wo_s, wr_s, wg_s, wu_s, wd_s,
            xn_s, wt_s, k_s, qt_s, vt_s, r_s, ot_s, o_s, out_s, xsel_s, act_s,
            sems, osems, *bufs):
    sa, sb = bufs[0:NQ], bufs[NQ:2 * NQ]
    ma, mb = bufs[2 * NQ:3 * NQ], bufs[3 * NQ:4 * NQ]

    cx = [pltpu.make_async_copy(x_hbm.at[pl.ds(i * RB, RB)], x_s.at[pl.ds(i * RB, RB)], sems.at[i])
          for i in range(NR)]
    cw = [pltpu.make_async_copy(w_hbm.at[:, pl.ds(j * D, D)], w_s.at[:, pl.ds(j * D, D)], sems.at[NR + j])
          for j in range(3)]
    cwr = pltpu.make_async_copy(wr_hbm, wr_s, sems.at[NR + 3])
    cwo = pltpu.make_async_copy(wo_hbm, wo_s, sems.at[NR + 4])
    cwg = pltpu.make_async_copy(wg_hbm, wg_s, sems.at[NR + 5])
    cwu = pltpu.make_async_copy(wu_hbm, wu_s, sems.at[NR + 6])
    cwd = pltpu.make_async_copy(wd_hbm, wd_s, sems.at[NR + 7])
    cx[0].start()
    cw[1].start()

    def layernorm(i):
        rows = slice(i * RB, (i + 1) * RB)
        xf = x_s[rows, :].astype(F32)
        mean = jnp.sum(xf, axis=1, keepdims=True) * (1.0 / D)
        cen = xf - mean
        var = jnp.sum(cen * cen, axis=1, keepdims=True) * (1.0 / D)
        t = _rb(_rb(var) + EPS_BF16)
        sd = _rb(t * lax.rsqrt(t))
        inv = pltpu.reciprocal(sd, approx=True)
        inv = inv * (2.0 - sd * inv)
        xn_s[rows, :] = (_rb(xf - _rb(mean)) * inv).astype(BF16)

    def proj_k(i):
        rows = slice(i * RB, (i + 1) * RB)
        k = jnp.dot(xn_s[rows, :], w_s[:, D:2 * D], preferred_element_type=F32).astype(BF16)
        for g in range(D // 128):
            k_s[g, rows, :] = k[:, g * 128:(g + 1) * 128]

    def proj_qv(i):
        rows = slice(i * RB, (i + 1) * RB)
        t = lax.dot_general(wt_s[...], xn_s[rows, :], (((1,), (1,)), ((), ())), preferred_element_type=F32)
        qt_s[:, rows] = (t[0:D] * QSCALE).astype(BF16)
        vt_s[:, rows] = t[D:2 * D].astype(BF16)
        r_s[:, rows] = t[2 * D:2 * D + 8]

    def weights_t():
        wt_s[0:D, :] = w_s[:, 0:D].T
        wt_s[D:2 * D, :] = w_s[:, 2 * D:3 * D].T
        wrow = lax.broadcasted_iota(jnp.int32, (16, D), 0)
        wr_f = jnp.broadcast_to(wr_s[...].astype(F32).reshape(1, D), (16, D))
        wt_s[2 * D:WROWS, :] = jnp.where(wrow == 0, wr_f, 0.0).astype(BF16)

    cx[0].wait()
    cx[1].start()
    cx[2].start()
    layernorm(0)
    cw[1].wait()
    cx[3].start()
    cw[0].start()
    cx[1].wait()
    cw[2].start()
    cwr.start()
    layernorm(1)
    proj_k(0)
    cx[2].wait()
    cx[3].wait()
    for i in range(4, NR):
        cx[i].start()
    layernorm(2)
    proj_k(1)
    layernorm(3)
    proj_k(2)
    cw[0].wait()
    cw[2].wait()
    cwr.wait()
    cwg.start()
    cwu.start()
    cwd.start()
    cwo.start()
    proj_k(3)
    weights_t()
    proj_qv(0)
    for i in range(4, NR):
        cx[i].wait()
    for i in range(1, NR):
        if i + 3 < NR:
            layernorm(i + 3)
        proj_qv(i)
        if i + 3 < NR:
            proj_k(i + 3)

    class RoutedFfn:
        def route(self):
            r = _rb(r_s[0:1, :])
            r = jnp.where(r != r, -jnp.inf, r)
            rmax = jnp.max(r, axis=1, keepdims=True)
            pos = lax.broadcasted_iota(jnp.int32, (1, S), 1)
            idx = jnp.min(jnp.where(r == rmax, pos, S - 1), axis=1, keepdims=True)[0, 0]
            self.base = pl.multiple_of((idx // 16) * 16, 16)
            self.sel = lax.broadcasted_iota(jnp.int32, (16, D), 0) == (idx - self.base)
            xblk = xn_s[pl.ds(self.base, 16), :].astype(F32)
            xsel_s[...] = jnp.where(self.sel, xblk, 0.0).astype(BF16)
            self.gain = jax.nn.sigmoid(rmax)

        def gate_up(self, j):
            cols = slice(j * FB, min((j + 1) * FB, F))
            xsel = xsel_s[...]
            gate = jnp.dot(xsel, wg_s[:, cols], preferred_element_type=F32)
            up = jnp.dot(xsel, wu_s[:, cols], preferred_element_type=F32)
            act_s[:, cols] = (gate * jax.nn.sigmoid(gate) * up).astype(BF16)

        def down(self, j):
            rows = slice(j * FB, min((j + 1) * FB, F))
            y = jnp.dot(act_s[:, rows], wd_s[rows, :], preferred_element_type=F32)
            self.y = y if j == 0 else self.y + y
            if (j + 1) * FB >= F:
                rows = pl.ds(self.base, 16)
                upd = jnp.where(self.sel, _rb(self.y * self.gain), 0.0)
                xn_s[rows, :] = (xn_s[rows, :].astype(F32) + upd).astype(BF16)

    ffn = RoutedFfn()
    def routed_ffn(u):
        if u == 0:
            ffn.route()
        elif T0 <= u < T0 + NF:
            ffn.gate_up(u - T0)
        elif T0 + NF + 2 <= u < T0 + 2 * NF + 2:
            ffn.down(u - T0 - NF - 2)

    class Pass1:
        def __init__(self, x, h, s_ref, m_ref):
            self.s_ref, self.m_ref = s_ref, m_ref
            self.g = h // HG
            q = qt_s[pl.ds(pl.multiple_of(self.g * 128, 128), 128), x * QB:(x + 1) * QB]
            q = pltpu.bitcast(q, jnp.uint32)
            row = lax.broadcasted_iota(jnp.int32, q.shape, 0)
            q = jnp.where((row >> 3) == h % HG, q, jnp.zeros_like(q))
            self.qm = pltpu.bitcast(q, BF16)
            self.mx = None

        def chunk(self, c):
            ks = slice(c * CH, (c + 1) * CH)
            s = jnp.dot(k_s[self.g, ks, :], self.qm, preferred_element_type=F32)
            self.s_ref[ks, :] = s
            cm = jnp.max(s.reshape(CH // 8, 8, QB), axis=0)
            self.mx = cm if self.mx is None else jnp.maximum(self.mx, cm)
            if c == NC - 1:
                self.m_ref[...] = jnp.max(self.mx, axis=0, keepdims=True)

    class Pass2:
        def __init__(self, x, h, s_ref, m_ref):
            self.x, self.s_ref, self.m_ref = x, s_ref, m_ref
            self.hrows = pl.ds(pl.multiple_of(h * DH, DH), DH)
            self.o = None
            self.l = None

        def chunk(self, c):
            ks = slice(c * CH, (c + 1) * CH)
            p = jnp.exp2(self.s_ref[ks, :] - self.m_ref[...])
            cl = None
            for j in reversed(range(CH // 8)):
                pj = p[j * 8:(j + 1) * 8, :]
                cl = pj if cl is None else cl + pj
            self.l = cl if self.l is None else self.l + cl
            co = jnp.dot(vt_s[self.hrows, ks], p.astype(BF16), preferred_element_type=F32)
            self.o = co if self.o is None else self.o + co
            if c == NC - 1:
                o = self.o / jnp.sum(self.l, axis=0, keepdims=True)
                ot_s[self.hrows, self.x * QB:(self.x + 1) * QB] = o.astype(BF16)

    def block(h1, s1, m1, h2, s2, m2, extra=None):
        units = []
        p1s, p2s = {}, {}
        for x in range(NQ):
            for c in range(NC):
                units.append((x, c))
        def do1(u):
            x, c = units[u]
            if c == 0:
                p1s[x] = Pass1(x, h1, s1[x], m1[x])
            p1s[x].chunk(c)
        def do2(u):
            x, c = units[u]
            if c == 0:
                p2s[x] = Pass2(x, h2, s2[x], m2[x])
            p2s[x].chunk(c)
        for u in range(len(units) + 1):
            if h2 is not None and u > 0:
                do2(u - 1)
            if u < len(units):
                do1(u)
            if extra is not None:
                extra(u)

    cwg.wait()
    cwu.wait()
    cwd.wait()
    block(0, sa, ma, None, None, None, routed_ffn)

    def head(i, carry):
        @pl.when(i % 2 == 0)
        def _():
            block(i + 1, sb, mb, i, sa, ma)

        @pl.when(i % 2 == 1)
        def _():
            block(i + 1, sa, ma, i, sb, mb)

        return carry

    lax.fori_loop(0, H - 1, head, 0)

    OB = 128
    NO = QB // OB
    outs = []

    def out_piece(x, j, n):
        if n == 0:
            cols = slice(x * QB + j * OB, x * QB + (j + 1) * OB)
            o_s[cols, :] = ot_s[:, cols].T
        rows = slice(x * QB + j * OB, x * QB + (j + 1) * OB)
        ns = slice(n * 128, (n + 1) * 128)
        a = jnp.dot(o_s[rows, :], wo_s[:, ns], preferred_element_type=F32)
        out_s[rows, ns] = (a + x_s[rows, ns].astype(F32) + xn_s[rows, ns].astype(F32)).astype(BF16)
        if j == NO - 1 and n == D // 128 - 1:
            cp = pltpu.make_async_copy(out_s.at[pl.ds(x * QB, QB)], out_hbm.at[pl.ds(x * QB, QB)], osems.at[x])
            cp.start()
            outs.append(cp)

    cwo.wait()
    for x in range(NQ):
        p2 = Pass2(x, H - 1, sb[x], mb[x])
        for c in range(NC):
            p2.chunk(c)
            if x > 0:
                out_piece(x - 1, c // (D // 128), c % (D // 128))
    for c in range(NC):
        out_piece(NQ - 1, c // (D // 128), c % (D // 128))
    for cp in outs:
        cp.wait()


@jax.jit
def pallas_parallel_sum__softmax_full_mha__moe_arch_mod__prompt_kernel(
    A_x: jax.Array,
    A_wqkv: jax.Array,
    A_wo: jax.Array,
    B_x: jax.Array,
    B_w_r: jax.Array,
    B_w_gate: jax.Array,
    B_w_up: jax.Array,
    B_w_down: jax.Array,
):
    del B_x
    any_spec = pl.BlockSpec(memory_space=pl.ANY)
    vmem = pltpu.VMEM
    scratch = [
        vmem((S, D), BF16),
        vmem((D, 3 * D), BF16),
        vmem((D, D), BF16),
        vmem((D,), BF16),
        vmem((D, F), BF16),
        vmem((D, F), BF16),
        vmem((F, D), BF16),
        vmem((S, D), BF16),
        vmem((WROWS, D), BF16),
        vmem((D // 128, S, 128), BF16),
        vmem((D, S), BF16),
        vmem((D, S), BF16),
        vmem((8, S), F32),
        vmem((D, S), BF16),
        vmem((S, D), BF16),
        vmem((S, D), BF16),
        vmem((16, D), BF16),
        vmem((16, F), BF16),
        pltpu.SemaphoreType.DMA((NR + 8,)),
        pltpu.SemaphoreType.DMA((NQ,)),
    ]
    scratch += [vmem((S, QB), F32)] * (2 * NQ)
    scratch += [vmem((1, QB), F32)] * (2 * NQ)
    out = pl.pallas_call(
        _kernel,
        out_shape=jax.ShapeDtypeStruct((S, D), A_x.dtype),
        in_specs=[any_spec] * 7,
        out_specs=any_spec,
        scratch_shapes=scratch,
        compiler_params=pltpu.CompilerParams(vmem_limit_bytes=100 * 1024 * 1024,
            flags={"XLA_TPU_EVENLY_DISTRIBUTE_CRITICAL_NODES": True}),
    )(A_x.reshape(S, D), A_wqkv, A_wo, B_w_r, B_w_gate, B_w_up, B_w_down)
    return out.reshape(1, S, D)
```

```python
import numpy as np
import jax
import jax.numpy as jnp
from jax import lax
import jax.experimental.pallas as pl
import jax.experimental.pallas.tpu as pltpu

S = 2048
D = 512
H = 32
DH = D // H
F = 1792

QB = 512
NQ = S // QB
CH = 128
NC = S // CH
RB = 256
NR = S // RB
HG = 128 // DH
FB = 128
NF = F // FB
T0 = 8
WROWS = 2 * D + 16

F32 = jnp.float32
BF16 = jnp.bfloat16
QSCALE = float(DH ** -0.5 * np.log2(np.e))
EPS_BF16 = float(np.asarray(1e-5, dtype=np.float32).astype(jnp.bfloat16).astype(np.float32))


def _rb(v):
    return v.astype(BF16).astype(F32)


def _kernel(x_hbm, w_hbm, wo_hbm, wr_hbm, wg_hbm, wu_hbm, wd_hbm, out_hbm,
            x_s, w_s, wo_s, wr_s, wg_s, wu_s, wd_s,
            xn_s, wt_s, k_s, qt_s, vt_s, r_s, ot_s, o_s, out_s, xsel_s, act_s,
            sems, osems, *bufs):
    sa, sb = bufs[0:NQ], bufs[NQ:2 * NQ]
    ma, mb = bufs[2 * NQ:3 * NQ], bufs[3 * NQ:4 * NQ]

    cx = [pltpu.make_async_copy(x_hbm.at[pl.ds(i * RB, RB)], x_s.at[pl.ds(i * RB, RB)], sems.at[i])
          for i in range(NR)]
    cw = [pltpu.make_async_copy(w_hbm.at[:, pl.ds(j * D, D)], w_s.at[:, pl.ds(j * D, D)], sems.at[NR + j])
          for j in range(3)]
    cwr = pltpu.make_async_copy(wr_hbm, wr_s, sems.at[NR + 3])
    cwo = pltpu.make_async_copy(wo_hbm, wo_s, sems.at[NR + 4])
    cwg = pltpu.make_async_copy(wg_hbm, wg_s, sems.at[NR + 5])
    cwu = pltpu.make_async_copy(wu_hbm, wu_s, sems.at[NR + 6])
    cwd = pltpu.make_async_copy(wd_hbm, wd_s, sems.at[NR + 7])
    cx[0].start()
    cw[1].start()

    def layernorm(i):
        rows = slice(i * RB, (i + 1) * RB)
        xf = x_s[rows, :].astype(F32)
        mean = jnp.sum(xf, axis=1, keepdims=True) * (1.0 / D)
        cen = xf - mean
        var = jnp.sum(cen * cen, axis=1, keepdims=True) * (1.0 / D)
        t = _rb(_rb(var) + EPS_BF16)
        sd = _rb(t * lax.rsqrt(t))
        inv = pltpu.reciprocal(sd, approx=True)
        inv = inv * (2.0 - sd * inv)
        xn_s[rows, :] = (_rb(xf - _rb(mean)) * inv).astype(BF16)

    def proj_k(i):
        rows = slice(i * RB, (i + 1) * RB)
        k = jnp.dot(xn_s[rows, :], w_s[:, D:2 * D], preferred_element_type=F32).astype(BF16)
        for g in range(D // 128):
            k_s[g, rows, :] = k[:, g * 128:(g + 1) * 128]

    def proj_qv(i):
        rows = slice(i * RB, (i + 1) * RB)
        t = lax.dot_general(wt_s[...], xn_s[rows, :], (((1,), (1,)), ((), ())), preferred_element_type=F32)
        qt_s[:, rows] = (t[0:D] * QSCALE).astype(BF16)
        vt_s[:, rows] = t[D:2 * D].astype(BF16)
        r_s[:, rows] = t[2 * D:2 * D + 8]

    def weights_t():
        wt_s[0:D, :] = w_s[:, 0:D].T
        wt_s[D:2 * D, :] = w_s[:, 2 * D:3 * D].T
        wrow = lax.broadcasted_iota(jnp.int32, (16, D), 0)
        wr_f = jnp.broadcast_to(wr_s[...].astype(F32).reshape(1, D), (16, D))
        wt_s[2 * D:WROWS, :] = jnp.where(wrow == 0, wr_f, 0.0).astype(BF16)

    cx[0].wait()
    cx[1].start()
    cx[2].start()
    layernorm(0)
    cw[1].wait()
    cx[3].start()
    cw[0].start()
    cx[1].wait()
    cw[2].start()
    cwr.start()
    layernorm(1)
    proj_k(0)
    cx[2].wait()
    cx[3].wait()
    for i in range(4, NR):
        cx[i].start()
    layernorm(2)
    proj_k(1)
    layernorm(3)
    proj_k(2)
    cw[0].wait()
    cw[2].wait()
    cwr.wait()
    cwg.start()
    cwu.start()
    cwd.start()
    cwo.start()
    proj_k(3)
    weights_t()
    proj_qv(0)
    for i in range(4, NR):
        cx[i].wait()
    for i in range(1, NR):
        if i + 3 < NR:
            layernorm(i + 3)
        proj_qv(i)
        if i + 3 < NR:
            proj_k(i + 3)

    class RoutedFfn:
        def route(self):
            r = _rb(r_s[0:1, :])
            r = jnp.where(r != r, -jnp.inf, r)
            rmax = jnp.max(r, axis=1, keepdims=True)
            pos = lax.broadcasted_iota(jnp.int32, (1, S), 1)
            idx = jnp.min(jnp.where(r == rmax, pos, S - 1), axis=1, keepdims=True)[0, 0]
            self.base = pl.multiple_of((idx // 16) * 16, 16)
            self.sel = lax.broadcasted_iota(jnp.int32, (16, D), 0) == (idx - self.base)
            xblk = xn_s[pl.ds(self.base, 16), :].astype(F32)
            xsel_s[...] = jnp.where(self.sel, xblk, 0.0).astype(BF16)
            self.gain = jax.nn.sigmoid(rmax)

        def gate_up(self, j):
            cols = slice(j * FB, min((j + 1) * FB, F))
            xsel = xsel_s[...]
            gate = jnp.dot(xsel, wg_s[:, cols], preferred_element_type=F32)
            up = jnp.dot(xsel, wu_s[:, cols], preferred_element_type=F32)
            act_s[:, cols] = (gate * jax.nn.sigmoid(gate) * up).astype(BF16)

        def down(self, j):
            rows = slice(j * FB, min((j + 1) * FB, F))
            y = jnp.dot(act_s[:, rows], wd_s[rows, :], preferred_element_type=F32)
            self.y = y if j == 0 else self.y + y
            if (j + 1) * FB >= F:
                rows = pl.ds(self.base, 16)
                upd = jnp.where(self.sel, _rb(self.y * self.gain), 0.0)
                xn_s[rows, :] = (xn_s[rows, :].astype(F32) + upd).astype(BF16)

    ffn = RoutedFfn()
    def routed_ffn(u):
        if u == 0:
            ffn.route()
        elif T0 <= u < T0 + NF:
            ffn.gate_up(u - T0)
        elif T0 + NF + 2 <= u < T0 + 2 * NF + 2:
            ffn.down(u - T0 - NF - 2)

    class Pass1:
        def __init__(self, x, h, s_ref, m_ref):
            self.s_ref, self.m_ref = s_ref, m_ref
            self.g = h // HG
            q = qt_s[pl.ds(pl.multiple_of(self.g * 128, 128), 128), x * QB:(x + 1) * QB]
            q = pltpu.bitcast(q, jnp.uint32)
            row = lax.broadcasted_iota(jnp.int32, q.shape, 0)
            q = jnp.where((row >> 3) == h % HG, q, jnp.zeros_like(q))
            self.qm = pltpu.bitcast(q, BF16)
            self.mx = None

        def chunk(self, c):
            ks = slice(c * CH, (c + 1) * CH)
            s = jnp.dot(k_s[self.g, ks, :], self.qm, preferred_element_type=F32)
            self.s_ref[ks, :] = s
            cm = jnp.max(s.reshape(CH // 8, 8, QB), axis=0)
            self.mx = cm if self.mx is None else jnp.maximum(self.mx, cm)
            if c == NC - 1:
                self.m_ref[...] = jnp.max(self.mx, axis=0, keepdims=True)

    class Pass2:
        def __init__(self, x, h, s_ref, m_ref):
            self.x, self.s_ref, self.m_ref = x, s_ref, m_ref
            self.hrows = pl.ds(pl.multiple_of(h * DH, DH), DH)
            self.o = None
            self.l = None

        def chunk(self, c):
            ks = slice(c * CH, (c + 1) * CH)
            p = jnp.exp2(self.s_ref[ks, :] - self.m_ref[...])
            cl = None
            for j in reversed(range(CH // 8)):
                pj = p[j * 8:(j + 1) * 8, :]
                cl = pj if cl is None else cl + pj
            self.l = cl if self.l is None else self.l + cl
            co = jnp.dot(vt_s[self.hrows, ks], p.astype(BF16), preferred_element_type=F32)
            self.o = co if self.o is None else self.o + co
            if c == NC - 1:
                o = self.o / jnp.sum(self.l, axis=0, keepdims=True)
                ot_s[self.hrows, self.x * QB:(self.x + 1) * QB] = o.astype(BF16)

    def block(h1, s1, m1, h2, s2, m2, extra=None):
        units = []
        p1s, p2s = {}, {}
        for x in range(NQ):
            for c in range(NC):
                units.append((x, c))
        def do1(u):
            x, c = units[u]
            if c == 0:
                p1s[x] = Pass1(x, h1, s1[x], m1[x])
            p1s[x].chunk(c)
        def do2(u):
            x, c = units[u]
            if c == 0:
                p2s[x] = Pass2(x, h2, s2[x], m2[x])
            p2s[x].chunk(c)
        for u in range(len(units) + 1):
            if h2 is not None and u > 0:
                do2(u - 1)
            if u < len(units):
                do1(u)
            if extra is not None:
                extra(u)

    cwg.wait()
    cwu.wait()
    cwd.wait()
    block(0, sa, ma, None, None, None, routed_ffn)

    def head(i, carry):
        block(2 * i + 1, sb, mb, 2 * i, sa, ma)

        @pl.when(i < H // 2 - 1)
        def _():
            block(2 * i + 2, sa, ma, 2 * i + 1, sb, mb)

        return carry

    lax.fori_loop(0, H // 2, head, 0)

    OB = 128
    NO = QB // OB
    outs = []

    def out_piece(x, j, n):
        if n == 0:
            cols = slice(x * QB + j * OB, x * QB + (j + 1) * OB)
            o_s[cols, :] = ot_s[:, cols].T
        rows = slice(x * QB + j * OB, x * QB + (j + 1) * OB)
        ns = slice(n * 128, (n + 1) * 128)
        a = jnp.dot(o_s[rows, :], wo_s[:, ns], preferred_element_type=F32)
        out_s[rows, ns] = (a + x_s[rows, ns].astype(F32) + xn_s[rows, ns].astype(F32)).astype(BF16)
        if n == D // 128 - 1:
            cp = pltpu.make_async_copy(out_s.at[rows], out_hbm.at[rows], osems.at[x * NO + j])
            cp.start()
            outs.append(cp)

    cwo.wait()
    for x in range(NQ):
        p2 = Pass2(x, H - 1, sb[x], mb[x])
        for c in range(NC):
            p2.chunk(c)
            if x > 0:
                out_piece(x - 1, c // (D // 128), c % (D // 128))
    for c in range(NC):
        out_piece(NQ - 1, c // (D // 128), c % (D // 128))
    for cp in outs:
        cp.wait()


@jax.jit
def pallas_parallel_sum__softmax_full_mha__moe_arch_mod__prompt_kernel(
    A_x: jax.Array,
    A_wqkv: jax.Array,
    A_wo: jax.Array,
    B_x: jax.Array,
    B_w_r: jax.Array,
    B_w_gate: jax.Array,
    B_w_up: jax.Array,
    B_w_down: jax.Array,
):
    del B_x
    any_spec = pl.BlockSpec(memory_space=pl.ANY)
    vmem = pltpu.VMEM
    scratch = [
        vmem((S, D), BF16),
        vmem((D, 3 * D), BF16),
        vmem((D, D), BF16),
        vmem((D,), BF16),
        vmem((D, F), BF16),
        vmem((D, F), BF16),
        vmem((F, D), BF16),
        vmem((S, D), BF16),
        vmem((WROWS, D), BF16),
        vmem((D // 128, S, 128), BF16),
        vmem((D, S), BF16),
        vmem((D, S), BF16),
        vmem((8, S), F32),
        vmem((D, S), BF16),
        vmem((S, D), BF16),
        vmem((S, D), BF16),
        vmem((16, D), BF16),
        vmem((16, F), BF16),
        pltpu.SemaphoreType.DMA((NR + 8,)),
        pltpu.SemaphoreType.DMA((S // 128,)),
    ]
    scratch += [vmem((S, QB), F32)] * (2 * NQ)
    scratch += [vmem((1, QB), F32)] * (2 * NQ)
    out = pl.pallas_call(
        _kernel,
        out_shape=jax.ShapeDtypeStruct((S, D), A_x.dtype),
        in_specs=[any_spec] * 7,
        out_specs=any_spec,
        scratch_shapes=scratch,
        compiler_params=pltpu.CompilerParams(vmem_limit_bytes=100 * 1024 * 1024,
            flags={"XLA_TPU_EVENLY_DISTRIBUTE_CRITICAL_NODES": True}),
    )(A_x.reshape(S, D), A_wqkv, A_wo, B_w_r, B_w_gate, B_w_up, B_w_down)
    return out.reshape(1, S, D)
```
